```python
import os as _os
_os.environ.setdefault('JAX_PLATFORMS', 'cpu')
import jax
import jax.numpy as jnp

def _softmax(x, axis=-1):
    return jax.nn.softmax(x, axis=axis)

def _gelu(x):
    return jax.nn.gelu(x, approximate=True)

def _silu(x):
    return jax.nn.silu(x)

def _sigmoid(x):
    return jax.nn.sigmoid(x)

def _layernorm(x, axis=-1, eps=1e-05):
    m = jnp.mean(x, axis=axis, keepdims=True)
    v = jnp.var(x, axis=axis, keepdims=True)
    return (x - m) / jnp.sqrt(v + eps)

def _scatter_add(tgt, idx, src, axis=0):
    return tgt.at[idx].add(src)

def _segment_sum(src, seg, n):
    return jax.ops.segment_sum(src, seg, n)

class _Rng:

    def __init__(self, key):
        self._k = key

    def _next(self):
        self._k, sub = jax.random.split(self._k)
        return sub

    def normal(self, shape):
        return jax.random.normal(self._next(), shape, dtype=jnp.bfloat16)

    def randint(self, lo, hi, shape):
        return jax.random.randint(self._next(), shape, lo, hi, dtype=jnp.int32)

    def uniform(self, shape, lo=0.0, hi=1.0):
        return jax.random.uniform(self._next(), shape, jnp.bfloat16, lo, hi)

    def permutation(self, n):
        return jax.random.permutation(self._next(), n)
kernel_name = 'parallel_sum__memory_aug_recurrent_mem_tr__dense_activation_gelu__prompt'

def setup_inputs():
    _rng = _Rng(jax.random.key(int.from_bytes(__import__("os").urandom(4), "little")))
    _w = lambda a: (lambda t: t.astype(jnp.bfloat16) if jnp.issubdtype(t.dtype, jnp.floating) else t)(jnp.asarray(a))

    def _A_setup():
        B, S, Dm = (1, 2048, 1024)
        H, Dh = (32, 128)
        M, seg = (8, 32)
        seg = min(seg, S)
        S = S // seg * seg
        return {'x': _w((lambda *s: _rng.normal(s) * 0.05)(B, S, Dm)), 'mem0': _w((lambda *s: _rng.normal(s) * 0.2)(B, M, Dm)), 'Wq': _w((lambda *s: _rng.normal(s) * 0.8)(Dm, H, Dh) * Dm ** (-0.5)), 'Wk': _w((lambda *s: _rng.normal(s) * 0.8)(Dm, H, Dh) * Dm ** (-0.5)), 'Wv': _w((lambda *s: _rng.normal(s) * 0.2)(Dm, H, Dh) * Dm ** (-0.5)), 'Wo': _w((lambda *s: _rng.normal(s) * 0.2)(H, Dh, Dm) * (H * Dh) ** (-0.5)), 'seg_len': seg}
    _A_in = _A_setup()

    def _B_setup():
        B, S, D, F = (1, 2048, 1024, 3584)
        return {'x': _w((lambda *s: _rng.normal(s) * 0.05)(B, S, D)), 'w1': _w((lambda *s: _rng.normal(s) * 0.1)(D, F) * D ** (-0.5)), 'b1': _w((lambda *s: _rng.normal(s) * 0.1)(F) * 0.01), 'w2': _w((lambda *s: _rng.normal(s) * 0.1)(F, D) * F ** (-0.5)), 'b2': _w((lambda *s: _rng.normal(s) * 0.05)(D) * 0.01)}
    _B_in = _B_setup()
    return {'A_x': _A_in['x'], 'A_mem0': _A_in['mem0'], 'A_Wq': _A_in['Wq'], 'A_Wk': _A_in['Wk'], 'A_Wv': _A_in['Wv'], 'A_Wo': _A_in['Wo'], 'A_seg_len': _A_in['seg_len'], 'B_x': _B_in['x'], 'B_w1': _B_in['w1'], 'B_b1': _B_in['b1'], 'B_w2': _B_in['w2'], 'B_b2': _B_in['b2']}

def reference(A_x, A_mem0, A_Wq, A_Wk, A_Wv, A_Wo, A_seg_len, B_x, B_w1, B_b1, B_w2, B_b2):

    def _A_ref(x, mem0, Wq, Wk, Wv, Wo, seg_len):
        B, S, Dm = x.shape
        H, Dh = (Wq.shape[1], Wq.shape[2])
        M = mem0.shape[1]
        scale = Dh ** (-0.5)
        n_seg = S // seg_len
        L = M + seg_len
        idx = jnp.arange(L)
        mask = (idx[:, None] < M) | (idx[:, None] >= idx[None, :])
        mem = mem0
        outs = []
        for s in range(n_seg):
            xs = x[:, s * seg_len:(s + 1) * seg_len, :].copy()
            h = jnp.concatenate([mem, xs], axis=1)
            q = jnp.einsum('btd,dhe->bhte', h, Wq)
            k = jnp.einsum('btd,dhe->bhte', h, Wk)
            v = jnp.einsum('btd,dhe->bhte', h, Wv)
            scores = jnp.einsum('bhqe,bhke->bhqk', q, k) * scale
            scores = jnp.where(mask[None, None], scores, -1000000000.0)
            p = _softmax(scores, axis=-1)
            o = jnp.einsum('bhqk,bhke->bhqe', p, v)
            o = jnp.einsum('bhte,hed->btd', o, Wo)
            mem = o[:, :M, :].copy()
            outs.append(o[:, M:, :])
        return jnp.concatenate(outs, axis=1)

    def _B_ref(x, w1, b1, w2, b2):
        h = jnp.einsum('bsd,df->bsf', x, w1) + b1
        h = _gelu(h)
        return jnp.einsum('bsf,fd->bsd', h, w2) + b2
    x = A_x
    xn = _layernorm(x, axis=-1)
    return x + _A_ref(xn, A_mem0, A_Wq, A_Wk, A_Wv, A_Wo, A_seg_len) + _B_ref(xn, B_w1, B_b1, B_w2, B_b2)
```

```python
import functools
import math

import jax
import jax.numpy as jnp
import numpy as np
from jax import lax
import jax.experimental.pallas as pl
import jax.experimental.pallas.tpu as pltpu

SKIP1 = int(0)
APPROX = int(1)
F32 = jnp.float32
BF16 = jnp.bfloat16
U32 = jnp.uint32


def _dot(a, b):
    return lax.dot_general(a, b, (((1,), (0,)), ((), ())), preferred_element_type=F32)


def _dot_nt(a, b):
    return lax.dot_general(a, b, (((1,), (1,)), ((), ())), preferred_element_type=F32)


def _kernel(x_hbm, mem0_ref, wq_hbm, wk_hbm, wv_hbm, wo_hbm, w1_hbm, b1_ref, w2_hbm, b2_ref,
            out_hbm,
            x_v, xn_v, acc_v, w1_v, w2_v, stg, wqkv, wo_v, hbuf, out_v, maskv, fillv, sems, osem,
            *, S, D, H, Dh, M, seg, F, RB, NC):
    L = M + seg
    n_seg = S // seg
    nrb = S // RB
    FC = F // NC
    HP = H // 2
    def cp_x(r):
        return pltpu.make_async_copy(x_hbm.at[pl.ds(r * RB, RB)], x_v.at[pl.ds(r * RB, RB)], sems.at[r])

    def cp_w1(c):
        return pltpu.make_async_copy(w1_hbm.at[:, pl.ds(c * FC, FC)], w1_v.at[c], sems.at[nrb + c])

    def cp_w2(c):
        return pltpu.make_async_copy(w2_hbm.at[pl.ds(c * FC, FC)], w2_v.at[c], sems.at[nrb + NC + c])

    whbm = (wq_hbm, wk_hbm, wv_hbm)

    def cp_w(i):
        return pltpu.make_async_copy(whbm[i], stg.at[i], sems.at[nrb + 2 * NC + i])

    def cp_wo(n):
        return pltpu.make_async_copy(wo_hbm.at[:, pl.ds(n * 128, 128)], wo_v.at[n], sems.at[nrb + 2 * NC + 3 + n])

    if not SKIP1:
        cp_x(0).start()
        cp_w1(0).start()
        cp_w2(0).start()
        for r in range(1, nrb):
            cp_x(r).start()

    b2 = b2_ref[...].astype(F32)

    FAKE = int(1)

    def relayout_unit(mi, u, zero):
        s32 = stg.at[mi].bitcast(U32)
        d0 = pl.multiple_of(u * 16, 16)
        X = s32[pl.ds(d0, 16)].reshape(8, 2, HP, Dh)
        A = X[:, 0]
        B = X[:, 1]
        E = (A & np.uint32(0xFFFF)) | (B << 16)
        O = (A >> 16) | (B & np.uint32(0xFFFF0000))
        Et = jnp.swapaxes(E, 0, 1)
        Ot = jnp.swapaxes(O, 0, 1)
        p0 = pl.multiple_of(u * 8, 8)
        z = None
        for j in range(HP):
            wqkv[mi, 2 * j, pl.ds(p0, 8), :] = Et[j]
            wqkv[mi, 2 * j + 1, pl.ds(p0, 8), :] = Ot[j]
            zz = Et[j] | Ot[j]
            z = zz if z is None else z | zz
        return pltpu.bitcast(z & zero, F32)

    n_units = D // 16

    def layernorm(r):
        r0 = pl.multiple_of(r * RB, RB)
        xf = x_v[pl.ds(r0, RB), :].astype(F32)
        m = jnp.mean(xf, axis=-1, keepdims=True)
        xc = xf - m
        var = jnp.mean(xc * xc, axis=-1, keepdims=True)
        xn = (xc * lax.rsqrt(var + 1e-5)).astype(BF16)
        xn_v[pl.ds(r0, RB), :] = xn
        return xn

    if not SKIP1:
        cp_x(0).wait()
        layernorm(0)

    for c in range(NC if not SKIP1 else 0):
        cp_w1(c).wait()
        if c + 1 < NC:
            cp_w1(c + 1).start()
            cp_w2(c + 1).start()
        if c < 3:
            cp_w(c).start()
        if c == 3:
            for n in range(D // 128):
                cp_wo(n).start()
        if c >= 1 and c <= 3:
            cp_w(c - 1).wait()
        b1c = b1_ref[:, c * FC:(c + 1) * FC].astype(F32)
        cp_w2(c).wait()

        def ffn_body(r, _, c=c, b1c=b1c):
            r0 = pl.multiple_of(r * RB, RB)
            zero = jnp.full((8, 128), r >> 20, jnp.int32).astype(U32)
            if c == 0:
                @pl.when(r + 1 < nrb)
                def _():
                    cp_x(r + 1).wait()
            xn = xn_v[pl.ds(r0, RB), :]
            hid = _dot(xn, w1_v[c]) + b1c
            hid = jax.nn.gelu(hid, approximate=True).astype(BF16)
            y = _dot(hid, w2_v[c])
            zs = None
            if c == 0:
                xn1 = layernorm(jnp.minimum(r + 1, nrb - 1))
                if FAKE:
                    xb = pltpu.bitcast(xn1, U32)
                    NT = D // 128
                    rows = RB // 2 // NT
                    zs = []
                    for n in range(NT):
                        blk = xb[n * rows:(n + 1) * rows]
                        z = None
                        for i in range(rows // 8):
                            for j in range(NT):
                                t = blk[i * 8:(i + 1) * 8, j * 128:(j + 1) * 128]
                                z = t if z is None else z | t
                        zs.append(pltpu.bitcast(z & zero, F32))
            elif c <= 3:
                upi = n_units // nrb
                zs = [relayout_unit(c - 1, r * upi + uu, zero) for uu in range(upi)]
                if not FAKE:
                    zs = None
                else:
                    NT = D // 128
                    per = upi // NT
                    zz = []
                    for n in range(NT):
                        z = zs[n * per]
                        for i in range(1, per):
                            z = z + zs[n * per + i]
                        zz.append(z)
                    zs = zz
            if zs is not None:
                y = jnp.concatenate([y[:8] + jnp.concatenate(zs, axis=1), y[8:]], axis=0)
            if c == 0:
                xf = x_v[pl.ds(r0, RB), :].astype(F32)
                acc_v[pl.ds(r0, RB), :] = y + (xf + b2)
            else:
                acc_v[pl.ds(r0, RB), :] += y
            return 0

        lax.fori_loop(0, nrb, ffn_body, 0)

    if not SKIP1:
        for n in range(D // 128):
            cp_wo(n).wait()

    ri = lax.broadcasted_iota(jnp.int32, (128, 128), 0)
    ci = lax.broadcasted_iota(jnp.int32, (128, 128), 1)
    rb_, rw = ri // L, ri % L
    cb_, cw = ci // L, ci % L
    same = (rb_ == cb_)
    valid_m = same & ((rw >= seg) | (cw >= seg) | (rw >= cw))
    log2e = math.log2(math.e)
    maskv[...] = valid_m.astype(F32)
    fillv[...] = jnp.where(same, -1e9 * log2e, -jnp.inf).astype(F32)
    cscale = (Dh ** -0.5) * log2e

    hbuf[pl.ds(seg, M), :] = mem0_ref[...].astype(F32)
    hbuf[pl.ds(0, seg), :] = xn_v[pl.ds(0, seg), :].astype(F32)

    def wtile(mi, h):
        return pltpu.bitcast(wqkv[mi, h], BF16)

    SGS = [[3,3,3,3],[3,3,3,3],[2,2,2,2]]
    sgs = []
    h0 = 0
    for sg in SGS:
        gl = []
        for gn in sg:
            gl.append((h0, gn)); h0 += gn
        sgs.append(gl)
    assert h0 == H
    NSG = len(sgs)
    KT = D // 128
    D1 = int(3)
    PVD = int(4)
    UNR = int(1)
    PVDL = int(4)

    def step(s):
        t0 = pl.multiple_of(s * seg, seg)
        hh = hbuf[...]
        q = {}; k = {}; v = {}; sc = {}; p = {}; o = {}; rl = {}
        outp = [None] * KT

        def do_q(h): q[h] = _dot(hh, wtile(0, h))
        def do_k(h): k[h] = _dot(hh, wtile(1, h))
        def do_v(h): v[h] = _dot(hh, wtile(2, h))
        def padcat(lst):
            n = sum(a.shape[0] for a in lst)
            return jnp.concatenate(lst + [jnp.zeros((128 - n, Dh), F32)], axis=0).astype(BF16)
        def do_s(g):
            g0, gn = g
            qq = jnp.concatenate([q[g0 + i] for i in range(gn)], axis=0)
            sc[g] = _dot_nt(qq, padcat([k[g0 + i] for i in range(gn)]))
        def do_sm(g):
            g0, gn = g
            R = gn * L
            t = jnp.where(maskv[0:R, :] > 0.5, sc[g] * cscale, fillv[0:R, :])
            mx = jnp.max(t, axis=-1, keepdims=True)
            pp = jnp.exp2(t - mx)
            l = jnp.sum(pp, axis=-1, keepdims=True)
            p[g] = pp
            r = pl.reciprocal(l, approx=True)
            rl[g] = r * (2.0 - l * r)
        def do_pv(g):
            g0, gn = g
            oo = _dot(p[g], padcat([v[g0 + i] for i in range(gn)])) * rl[g]
            for i in range(gn):
                o[g0 + i] = oo[i * L:(i + 1) * L]
        def do_wo(si, n):
            hs = [g0 + i for (g0, gn) in sgs[si] for i in range(gn)]
            oc = jnp.concatenate([o[h] for h in hs], axis=1)
            r = _dot(oc, wo_v[n, hs[0] * Dh:(hs[-1] + 1) * Dh, :])
            outp[n] = r if outp[n] is None else r + outp[n]
        def do_next_tokens():
            s1 = jnp.minimum(s + 1, n_seg - 1)
            hbuf[pl.ds(0, seg), :] = xn_v[pl.ds(pl.multiple_of(s1 * seg, seg), seg), :].astype(F32)

        tasks = []
        def heads(si): return [g0 + i for (g0, gn) in sgs[si] for i in range(gn)]
        pending = []
        for si in range(NSG):
            main = []
            for h in heads(si):
                main.append(lambda h=h: do_q(h))
                main.append(lambda h=h: do_k(h))
            vlist = [(lambda h=h: do_v(h)) for h in heads(si)]
            main += vlist[:D1]
            for g in sgs[si]:
                main.append(lambda g=g: do_s(g))
            for g in sgs[si]:
                main.append(lambda g=g: do_sm(g))
            main += vlist[D1:]
            if pending:
                main = main[:PVD] + pending + main[PVD:]
            pending = [(lambda g=g: do_pv(g)) for g in sgs[si]]
            tasks += main
        tasks.append(do_next_tokens)
        wo_tasks = []
        for si in range(NSG):
            for n in range(KT):
                wo_tasks.append(lambda si=si, n=n: do_wo(si, n))
        tasks += wo_tasks[:PVDL] + pending + wo_tasks[PVDL:]
        for t in tasks:
            t()
        res = jnp.concatenate(outp, axis=1)
        hbuf[pl.ds(seg, M), :] = res[seg:]
        out_v[pl.ds(t0, seg), :] = (acc_v[pl.ds(t0, seg), :] + res[:seg]).astype(BF16)

    def stepu(i, _):
        for u in range(UNR):
            step(i * UNR + u)
        return 0

    OB = 256
    spb = OB // seg

    def cp_out(b):
        return pltpu.make_async_copy(out_v.at[pl.ds(b * OB, OB)], out_hbm.at[pl.ds(b * OB, OB)], osem.at[0])

    def outer(b, _):
        lax.fori_loop(b * (spb // UNR), (b + 1) * (spb // UNR), stepu, 0)
        pltpu.make_async_copy(out_v.at[pl.ds(pl.multiple_of(b * OB, OB), OB)],
                              out_hbm.at[pl.ds(pl.multiple_of(b * OB, OB), OB)], osem.at[0]).start()
        return 0

    lax.fori_loop(0, int(S // OB), outer, 0)
    for b in range(int(S // OB)):
        cp_out(b).wait()


@functools.partial(jax.jit, static_argnames=("A_seg_len",))
def pallas_parallel_sum__memory_aug_recurrent_mem_tr__dense_activation_gelu__prompt_kernel(
    A_x, A_mem0, A_Wq, A_Wk, A_Wv, A_Wo, A_seg_len, B_x, B_w1, B_b1, B_w2, B_b2,
):
    del B_x
    _, S, D = A_x.shape
    _, H, Dh = A_Wq.shape
    M = A_mem0.shape[1]
    seg = int(A_seg_len)
    F = B_w1.shape[1]
    RB = 256
    NC = 4
    FC = F // NC
    nrb = S // RB
    kern = functools.partial(_kernel, S=S, D=D, H=H, Dh=Dh, M=M, seg=seg, F=F, RB=RB, NC=NC)
    hbm = pl.BlockSpec(memory_space=pl.ANY)
    vm = pl.BlockSpec(memory_space=pltpu.VMEM)
    out = pl.pallas_call(
        kern,
        out_shape=jax.ShapeDtypeStruct((S, D), BF16),
        in_specs=[hbm, vm, hbm, hbm, hbm, hbm, hbm, vm, hbm, vm],
        out_specs=hbm,
        scratch_shapes=[
            pltpu.VMEM((S, D), BF16),
            pltpu.VMEM((S, D), BF16),
            pltpu.VMEM((S, D), F32),
            pltpu.VMEM((NC, D, FC), BF16),
            pltpu.VMEM((NC, FC, D), BF16),
            pltpu.VMEM((3, D, H, Dh), BF16),
            pltpu.VMEM((3, H, D // 2, Dh), U32),
            pltpu.VMEM((D // 128, H * Dh, 128), BF16),
            pltpu.VMEM((M + seg, D), F32),
            pltpu.VMEM((S, D), BF16),
            pltpu.VMEM((128, 128), F32),
            pltpu.VMEM((128, 128), F32),
            pltpu.SemaphoreType.DMA((nrb + 2 * NC + 3 + D // 128,)),
            pltpu.SemaphoreType.DMA((1,)),
        ],
        compiler_params=pltpu.CompilerParams(vmem_limit_bytes=110 * 1024 * 1024),
    )(A_x.reshape(S, D), A_mem0.reshape(M, D), A_Wq, A_Wk, A_Wv, A_Wo.reshape(H * Dh, D),
      B_w1, B_b1.reshape(1, F), B_w2, B_b2.reshape(1, D))
    return out.reshape(1, S, D)
```

```python
import functools
import math

import jax
import jax.numpy as jnp
import numpy as np
from jax import lax
import jax.experimental.pallas as pl
import jax.experimental.pallas.tpu as pltpu

F32 = jnp.float32
BF16 = jnp.bfloat16
U32 = jnp.uint32
LANES = 128


def _dot(a, b):
    return lax.dot_general(a, b, (((1,), (0,)), ((), ())), preferred_element_type=F32)


def _dot_nt(a, b):
    return lax.dot_general(a, b, (((1,), (1,)), ((), ())), preferred_element_type=F32)


def _unrolled_loop(n, unroll, body):
    unroll = unroll if n % unroll == 0 else 1

    def f(i, carry):
        for k in range(unroll):
            body(i * unroll + k)
        return carry

    lax.fori_loop(0, n // unroll, f, 0)


def _kernel(x_hbm, mem0_hbm, wq_hbm, wk_hbm, wv_hbm, wo_hbm, w1_hbm, b1_hbm, w2_hbm, b2_hbm,
            out_hbm,
            x_v, xn_v, acc_v, w1a_v, w2a_v, w1s_v, w2s_v, bias_v, stg, wqkv, wo_v,
            hbuf, out_v, maskv, fillv, mem0_v, b1_v, b2_v, sems, osem,
            *, S, D, H, Dh, M, seg, F, RB, NA, NS, groups):
    L = M + seg
    n_seg = S // seg
    nrb = S // RB
    HP = H // 2
    KT = D // LANES
    coff = [0] + [NA + k * NS for k in range(4)]
    w1_dst = [w1a_v] + [w1s_v.at[k] for k in range(3)]
    w2_dst = [w2a_v] + [w2s_v.at[k] for k in range(3)]

    s_x, s_w1, s_w2, s_w, s_wo = 0, nrb, nrb + 4, nrb + 8, nrb + 11
    s_mem, s_b1, s_b2 = s_wo + KT, s_wo + KT + 1, s_wo + KT + 2

    def cp_x(r):
        r0 = r * RB if isinstance(r, int) else pl.multiple_of(r * RB, RB)
        return pltpu.make_async_copy(x_hbm.at[pl.ds(r0, RB)], x_v.at[pl.ds(r0, RB)], sems.at[s_x + r])

    def cp_w1(c):
        return pltpu.make_async_copy(w1_hbm.at[:, pl.ds(coff[c], coff[c + 1] - coff[c])], w1_dst[c],
                                     sems.at[s_w1 + c])

    def cp_w2(c):
        return pltpu.make_async_copy(w2_hbm.at[pl.ds(coff[c], coff[c + 1] - coff[c])], w2_dst[c],
                                     sems.at[s_w2 + c])

    whbm = (wq_hbm, wk_hbm, wv_hbm)

    def cp_w(i):
        return pltpu.make_async_copy(whbm[i], stg.at[i], sems.at[s_w + i])

    def cp_wo(n):
        return pltpu.make_async_copy(wo_hbm.at[:, pl.ds(n * LANES, LANES)], wo_v.at[n], sems.at[s_wo + n])

    cp_mem = pltpu.make_async_copy(mem0_hbm, mem0_v, sems.at[s_mem])
    cp_b1 = pltpu.make_async_copy(b1_hbm, b1_v, sems.at[s_b1])
    cp_b2 = pltpu.make_async_copy(b2_hbm, b2_v, sems.at[s_b2])

    cp_x(0).start()
    cp_w1(0).start()
    cp_b1.start()
    cp_b2.start()
    cp_w2(0).start()
    for r in range(1, nrb):
        cp_x(r).start()
    cp_mem.start()

    ri = lax.broadcasted_iota(jnp.int32, (LANES, LANES), 0)
    ci = lax.broadcasted_iota(jnp.int32, (LANES, LANES), 1)
    rb_, rw = ri // L, ri % L
    cb_, cw = ci // L, ci % L
    same = rb_ == cb_
    valid = same & ((rw >= seg) | (cw >= seg) | (rw >= cw))
    log2e = math.log2(math.e)
    maskv[...] = valid.astype(F32)
    fillv[...] = jnp.where(same, -1e9 * log2e, -jnp.inf).astype(F32)
    cscale = (Dh ** -0.5) * log2e

    def relayout_unit(mi, u, zero):
        s32 = stg.at[mi].bitcast(U32)
        d0 = pl.multiple_of(u * 16, 16)
        X = s32[pl.ds(d0, 16)].reshape(8, 2, HP, Dh)
        A = X[:, 0]
        B = X[:, 1]
        E = (A & np.uint32(0xFFFF)) | (B << 16)
        O = (A >> 16) | (B & np.uint32(0xFFFF0000))
        Et = jnp.swapaxes(E, 0, 1)
        Ot = jnp.swapaxes(O, 0, 1)
        p0 = pl.multiple_of(u * 8, 8)
        z = None
        for j in range(HP):
            wqkv[mi, 2 * j, pl.ds(p0, 8), :] = Et[j]
            wqkv[mi, 2 * j + 1, pl.ds(p0, 8), :] = Ot[j]
            zz = Et[j] | Ot[j]
            z = zz if z is None else z | zz
        return pltpu.bitcast(z & zero, F32)

    def layernorm(r):
        r0 = pl.multiple_of(r * RB, RB)
        xf = x_v[pl.ds(r0, RB), :].astype(F32)
        m = jnp.mean(xf, axis=-1, keepdims=True)
        xc = xf - m
        var = jnp.mean(xc * xc, axis=-1, keepdims=True)
        xn = (xc * lax.rsqrt(var + 1e-5)).astype(BF16)
        xn_v[pl.ds(r0, RB), :] = xn
        return xn

    def opaque_zero(r):
        return jnp.full((8, LANES), r >> 20, jnp.int32).astype(U32)

    def ffn_block(r, w1, w2, bias, side_work, first):
        r0 = pl.multiple_of(r * RB, RB)
        xn = xn_v[pl.ds(r0, RB), :]
        hid = _dot(xn, w1) + bias
        hid = jax.nn.gelu(hid, approximate=True).astype(BF16)
        y = _dot(hid, w2)
        zs = side_work()
        y = jnp.concatenate([y[:8] + jnp.concatenate(zs, axis=1), y[8:]], axis=0)
        if first:
            xf = x_v[pl.ds(r0, RB), :].astype(F32)
            acc_v[pl.ds(r0, RB), :] = y + (xf + b2)
        else:
            acc_v[pl.ds(r0, RB), :] += y

    cp_x(0).wait()
    layernorm(0)
    cp_w1(0).wait()
    cp_b1.wait()
    cp_b2.wait()
    b1 = b1_v[...].astype(F32).reshape(1, F)
    b2 = b2_v[...].astype(F32).reshape(1, D)
    for k in range(3):
        bias_v[k] = jnp.broadcast_to(b1[:, coff[1 + k]:coff[2 + k]], (8, NS))

    cp_w1(1).start()
    cp_w2(1).start()
    cp_w(0).start()
    cp_w2(0).wait()

    def first_chunk(r):
        @pl.when(r + 1 < nrb)
        def _():
            cp_x(r + 1).wait()

        def next_layernorm():
            zero = opaque_zero(r)
            xb = pltpu.bitcast(layernorm(jnp.minimum(r + 1, nrb - 1)), U32)
            rows = RB // 2 // KT
            zs = []
            for n in range(KT):
                blk = xb[n * rows:(n + 1) * rows]
                z = None
                for i in range(rows // 8):
                    for j in range(KT):
                        t = blk[i * 8:(i + 1) * 8, j * LANES:(j + 1) * LANES]
                        z = t if z is None else z | t
                zs.append(pltpu.bitcast(z & zero, F32))
            return zs

        ffn_block(r, w1a_v[...], w2a_v[...], b1[:, coff[0]:coff[1]], next_layernorm, True)

    _unrolled_loop(nrb, 1, first_chunk)

    n_units = D // 16

    def later_chunk(k, carry):
        for kk in range(3):
            @pl.when(k == kk)
            def _(kk=kk):
                cp_w1(1 + kk).wait()
                if kk < 2:
                    cp_w1(2 + kk).start()
                    cp_w2(2 + kk).start()
                    cp_w(kk + 1).start()
                else:
                    for n in range(KT):
                        cp_wo(n).start()
                cp_w(kk).wait()
                cp_w2(1 + kk).wait()

        def body(r):
            def relayout():
                zero = opaque_zero(r)
                upi = n_units // nrb
                zu = [relayout_unit(k, r * upi + uu, zero) for uu in range(upi)]
                per = upi // KT
                zs = []
                for n in range(KT):
                    z = zu[n * per]
                    for i in range(1, per):
                        z = z + zu[n * per + i]
                    zs.append(z)
                return zs

            ffn_block(r, w1s_v[k], w2s_v[k], bias_v[k, 0:1, :], relayout, False)

        _unrolled_loop(nrb, 2, body)
        return carry

    lax.fori_loop(0, 3, later_chunk, 0)

    for n in range(KT):
        cp_wo(n).wait()
    cp_mem.wait()

    hbuf[pl.ds(seg, M), :] = mem0_v[...].astype(F32)
    hbuf[pl.ds(0, seg), :] = xn_v[pl.ds(0, seg), :].astype(F32)

    def wtile(mi, h):
        return pltpu.bitcast(wqkv[mi, h], BF16)

    sgs, h0 = [], 0
    for sg in groups:
        gl = []
        for gn in sg:
            gl.append((h0, gn))
            h0 += gn
        sgs.append(gl)
    assert h0 == H
    NSG = len(sgs)
    V_BEFORE_S = 3
    PV_DELAY = 4
    N_SPLIT = 2
    UNROLL = 4 if n_seg % 4 == 0 else 1

    def cp_out(s):
        t0 = s * seg if isinstance(s, int) else pl.multiple_of(s * seg, seg)
        return pltpu.make_async_copy(out_v.at[pl.ds(t0, seg)], out_hbm.at[pl.ds(t0, seg)], osem.at[0])

    def step(s):
        t0 = pl.multiple_of(s * seg, seg)
        hh = hbuf[...]
        q, k, v, sc, p, rl, o = {}, {}, {}, {}, {}, {}, {}
        outp = [None] * KT

        def do_q(h):
            q[h] = _dot(hh, wtile(0, h))

        def do_k(h):
            k[h] = _dot(hh, wtile(1, h))

        def do_v(h):
            v[h] = _dot(hh, wtile(2, h))

        def half(mi, h, part):
            HD = D // 2
            w = pltpu.bitcast(wqkv[mi, h, part * (HD // 2):(part + 1) * (HD // 2), :], BF16)
            return _dot(hh[:, part * HD:(part + 1) * HD], w)

        def do_first(hs):
            qa = {h: half(0, h, 0) for h in hs}
            ka = {h: half(1, h, 0) for h in hs}
            for h in hs:
                q[h] = half(0, h, 1) + qa[h]
                k[h] = half(1, h, 1) + ka[h]

        def padcat(lst):
            n = sum(a.shape[0] for a in lst)
            return jnp.concatenate(lst + [jnp.zeros((LANES - n, Dh), F32)], axis=0).astype(BF16)

        def do_s(g):
            g0, gn = g
            qq = jnp.concatenate([q[g0 + i] for i in range(gn)], axis=0)
            sc[g] = _dot_nt(qq, padcat([k[g0 + i] for i in range(gn)]))

        def do_softmax(g):
            g0, gn = g
            R = gn * L
            t = jnp.where(maskv[0:R, :] > 0.5, sc[g] * cscale, fillv[0:R, :])
            mx = jnp.max(t, axis=-1, keepdims=True)
            pp = jnp.exp2(t - mx)
            l = jnp.sum(pp, axis=-1, keepdims=True)
            p[g] = pp
            r = pl.reciprocal(l, approx=True)
            rl[g] = r * (2.0 - l * r)

        def do_pv(g):
            g0, gn = g
            oo = _dot(p[g], padcat([v[g0 + i] for i in range(gn)])) * rl[g]
            for i in range(gn):
                o[g0 + i] = oo[i * L:(i + 1) * L]

        def heads(si):
            return [g0 + i for (g0, gn) in sgs[si] for i in range(gn)]

        def do_wo(si, n):
            hs = heads(si)
            oc = jnp.concatenate([o[h] for h in hs], axis=1)
            r = _dot(oc, wo_v[n, hs[0] * Dh:(hs[-1] + 1) * Dh, :])
            outp[n] = r if outp[n] is None else r + outp[n]

        def do_next_tokens():
            s1 = jnp.minimum(s + 1, n_seg - 1)
            hbuf[pl.ds(0, seg), :] = xn_v[pl.ds(pl.multiple_of(s1 * seg, seg), seg), :].astype(F32)

        tasks, pending = [], []
        for si in range(NSG):
            main = []
            hl = heads(si)
            if si == 0:
                main.append(functools.partial(do_first, hl[:N_SPLIT]))
                hl = hl[N_SPLIT:]
            for h in hl:
                main.append(functools.partial(do_q, h))
                main.append(functools.partial(do_k, h))
            vlist = [functools.partial(do_v, h) for h in heads(si)]
            main += vlist[:V_BEFORE_S]
            main += [functools.partial(do_s, g) for g in sgs[si]]
            main += [functools.partial(do_softmax, g) for g in sgs[si]]
            main += vlist[V_BEFORE_S:]
            if pending:
                main = main[:PV_DELAY] + pending + main[PV_DELAY:]
            pending = [functools.partial(do_pv, g) for g in sgs[si]]
            tasks += main
        tasks.append(do_next_tokens)
        wo_tasks = [functools.partial(do_wo, si, n) for si in range(NSG) for n in range(KT)]
        tasks += wo_tasks[:PV_DELAY] + pending + wo_tasks[PV_DELAY:]
        for t in tasks:
            t()
        res = jnp.concatenate(outp, axis=1)
        hbuf[pl.ds(seg, M), :] = res[seg:]
        out_v[pl.ds(t0, seg), :] = (acc_v[pl.ds(t0, seg), :] + res[:seg]).astype(BF16)

    def steps(i, carry):
        @pl.when(i > 0)
        def _():
            cp_out(i * UNROLL - 1).start()

        for u in range(UNROLL):
            if u > 0:
                cp_out(i * UNROLL + u - 1).start()
            step(i * UNROLL + u)
        return carry

    lax.fori_loop(0, n_seg // UNROLL, steps, 0)
    cp_out(n_seg - 1).start()
    for s in range(n_seg):
        cp_out(s).wait()


@functools.partial(jax.jit, static_argnames=("A_seg_len",))
def pallas_parallel_sum__memory_aug_recurrent_mem_tr__dense_activation_gelu__prompt_kernel(
    A_x, A_mem0, A_Wq, A_Wk, A_Wv, A_Wo, A_seg_len, B_x, B_w1, B_b1, B_w2, B_b2,
):
    del B_x
    _, S, D = A_x.shape
    _, H, Dh = A_Wq.shape
    M = A_mem0.shape[1]
    seg = int(A_seg_len)
    F = B_w1.shape[1]
    RB = 256
    NS = (F // LANES * 2 // 7) * LANES
    NA = F - 3 * NS
    groups = ((2, 2, 2, 2), (3, 3, 3, 3), (3, 3, 3, 3))
    assert Dh == LANES and 3 * (M + seg) <= LANES and sum(map(sum, groups)) == H
    nrb = S // RB
    kern = functools.partial(_kernel, S=S, D=D, H=H, Dh=Dh, M=M, seg=seg, F=F, RB=RB, NA=NA, NS=NS,
                             groups=groups)
    hbm = pl.BlockSpec(memory_space=pl.ANY)
    out = pl.pallas_call(
        kern,
        out_shape=jax.ShapeDtypeStruct((S, D), BF16),
        in_specs=[hbm] * 10,
        out_specs=hbm,
        scratch_shapes=[
            pltpu.VMEM((S, D), BF16),
            pltpu.VMEM((S, D), BF16),
            pltpu.VMEM((S, D), F32),
            pltpu.VMEM((D, NA), BF16),
            pltpu.VMEM((NA, D), BF16),
            pltpu.VMEM((3, D, NS), BF16),
            pltpu.VMEM((3, NS, D), BF16),
            pltpu.VMEM((3, 8, NS), F32),
            pltpu.VMEM((3, D, H, Dh), BF16),
            pltpu.VMEM((3, H, D // 2, Dh), U32),
            pltpu.VMEM((D // LANES, H * Dh, LANES), BF16),
            pltpu.VMEM((M + seg, D), F32),
            pltpu.VMEM((S, D), BF16),
            pltpu.VMEM((LANES, LANES), F32),
            pltpu.VMEM((LANES, LANES), F32),
            pltpu.VMEM((M, D), BF16),
            pltpu.VMEM((F,), BF16),
            pltpu.VMEM((D,), BF16),
            pltpu.SemaphoreType.DMA((nrb + 11 + D // LANES + 3,)),
            pltpu.SemaphoreType.DMA((1,)),
        ],
        compiler_params=pltpu.CompilerParams(vmem_limit_bytes=110 * 1024 * 1024),
    )(A_x.reshape(S, D), A_mem0.reshape(M, D), A_Wq, A_Wk, A_Wv, A_Wo.reshape(H * Dh, D),
      B_w1, B_b1, B_w2, B_b2)
    return out.reshape(1, S, D)
```

```python
import functools
import math

import jax
import jax.numpy as jnp
import numpy as np
from jax import lax
import jax.experimental.pallas as pl
import jax.experimental.pallas.tpu as pltpu

F32 = jnp.float32
BF16 = jnp.bfloat16
U32 = jnp.uint32
LANES = 128
_reciprocal = pltpu.reciprocal if hasattr(pltpu, "reciprocal") else pl.reciprocal


def _dot(a, b):
    return lax.dot_general(a, b, (((1,), (0,)), ((), ())), preferred_element_type=F32)


def _dot_nt(a, b):
    return lax.dot_general(a, b, (((1,), (1,)), ((), ())), preferred_element_type=F32)


def _unrolled_loop(n, unroll, body):
    unroll = unroll if n % unroll == 0 else 1

    def f(i, carry):
        for k in range(unroll):
            body(i * unroll + k)
        return carry

    lax.fori_loop(0, n // unroll, f, 0)


def _kernel(x_hbm, mem0_hbm, wq_hbm, wk_hbm, wv_hbm, wo_hbm, w1_hbm, b1_hbm, w2_hbm, b2_hbm,
            out_hbm,
            x_v, xn_v, acc_v, w1a_v, w2a_v, w1s_v, w2s_v, biasa_v, bias_v, stg, wqkv, wo_v,
            hbuf, out_v, maskv, fillv, mem0_v, b1_v, b2_v, sems, osem,
            *, S, D, H, Dh, M, seg, F, RB, NA, NS, groups):
    L = M + seg
    n_seg = S // seg
    nrb = S // RB
    HP = H // 2
    KT = D // LANES
    n_units = D // 16

    s_small = nrb
    s_tile = nrb + 1
    NTA = NA // LANES

    def cp_x(r):
        r0 = r * RB if isinstance(r, int) else pl.multiple_of(r * RB, RB)
        return pltpu.make_async_copy(x_hbm.at[pl.ds(r0, RB)], x_v.at[pl.ds(r0, RB)], sems.at[r])

    def cp_t1(j):
        sl = pl.ds(j * LANES, LANES)
        return pltpu.make_async_copy(w1_hbm.at[:, sl], w1a_v.at[:, sl], sems.at[s_tile + j])

    def cp_t2(j):
        sl = pl.ds(j * LANES, LANES)
        return pltpu.make_async_copy(w2_hbm.at[sl], w2a_v.at[sl], sems.at[s_tile + j])

    def chunk_sem(k):
        return sems.at[s_tile + k % 2]

    whbm = (wq_hbm, wk_hbm, wv_hbm)

    def cp_chunk(k):
        sl = pl.ds(NA + k * NS, NS)
        return [pltpu.make_async_copy(w1_hbm.at[:, sl], w1s_v.at[k], chunk_sem(k)),
                pltpu.make_async_copy(w2_hbm.at[sl], w2s_v.at[k], chunk_sem(k)),
                pltpu.make_async_copy(whbm[k], stg.at[k], chunk_sem(k))]

    cp_wo = [pltpu.make_async_copy(wo_hbm.at[:, pl.ds(n * LANES, LANES)], wo_v.at[n], chunk_sem(3))
             for n in range(KT)]
    cp_small = [pltpu.make_async_copy(src, dst, sems.at[s_small])
                for src, dst in ((b1_hbm, b1_v), (b2_hbm, b2_v), (mem0_hbm, mem0_v))]

    cp_x(0).start()
    cp_x(1).start()
    for cp in cp_small:
        cp.start()
    for j in range(NTA):
        cp_t1(j).start()
        cp_t2(j).start()
    for r in range(2, nrb):
        cp_x(r).start()

    ri = lax.broadcasted_iota(jnp.int32, (LANES, LANES), 0)
    ci = lax.broadcasted_iota(jnp.int32, (LANES, LANES), 1)
    rb_ = (ri >= L).astype(jnp.int32) + (ri >= 2 * L) + (ri >= 3 * L)
    cb_ = (ci >= L).astype(jnp.int32) + (ci >= 2 * L) + (ci >= 3 * L)
    rw, cw = ri - L * rb_, ci - L * cb_
    same = rb_ == cb_
    valid = same & ((rw >= seg) | (cw >= seg) | (rw >= cw))
    log2e = math.log2(math.e)
    maskv[...] = valid.astype(F32)
    fillv[...] = jnp.where(same, -1e9 * log2e, -jnp.inf).astype(F32)
    cscale = (Dh ** -0.5) * log2e

    def relayout_unit(mi, u, zero):
        s32 = stg.at[mi].bitcast(U32)
        d0 = pl.multiple_of(u * 16, 16)
        X = s32[pl.ds(d0, 16)].reshape(8, 2, HP, Dh)
        A = X[:, 0]
        B = X[:, 1]
        E = (A & np.uint32(0xFFFF)) | (B << 16)
        O = (A >> 16) | (B & np.uint32(0xFFFF0000))
        Et = jnp.swapaxes(E, 0, 1)
        Ot = jnp.swapaxes(O, 0, 1)
        p0 = pl.multiple_of(u * 8, 8)
        z = None
        for j in range(HP):
            wqkv[mi, 2 * j, pl.ds(p0, 8), :] = Et[j]
            wqkv[mi, 2 * j + 1, pl.ds(p0, 8), :] = Ot[j]
            zz = Et[j] | Ot[j]
            z = zz if z is None else z | zz
        return pltpu.bitcast(z & zero, F32)

    def layernorm(r):
        r0 = pl.multiple_of(r * RB, RB)
        xf = x_v[pl.ds(r0, RB), :].astype(F32)
        m = jnp.mean(xf, axis=-1, keepdims=True)
        xc = xf - m
        var = jnp.mean(xc * xc, axis=-1, keepdims=True)
        xn = (xc * lax.rsqrt(var + 1e-5)).astype(BF16)
        xn_v[pl.ds(r0, RB), :] = xn
        return xn

    def opaque_zero(r):
        return jnp.full((8, LANES), r >> 20, jnp.int32).astype(U32)

    def ffn_block(r, w1, w2, bias, side_work, first):
        r0 = pl.multiple_of(r * RB, RB)
        xn = xn_v[pl.ds(r0, RB), :]
        hid = _dot(xn, w1) + bias
        hid = jax.nn.gelu(hid, approximate=True).astype(BF16)
        y = _dot(hid, w2)
        zs = side_work()
        y = jnp.concatenate([y[:8] + jnp.concatenate(zs, axis=1), y[8:]], axis=0)
        if first:
            xf = x_v[pl.ds(r0, RB), :].astype(F32)
            acc_v[pl.ds(r0, RB), :] = y + (xf + b2)
        else:
            acc_v[pl.ds(r0, RB), :] += y

    def first_layernorms(r, carry):
        for rr in range(2):
            @pl.when(r == rr)
            def _(rr=rr):
                cp_x(rr).wait()
        layernorm(r)
        return carry

    lax.fori_loop(0, 2, first_layernorms, 0)
    for cp in cp_small:
        cp.wait()
    b1 = b1_v[...].astype(F32).reshape(1, F)
    b2 = b2_v[...].astype(F32).reshape(1, D)
    biasa_v[...] = jnp.broadcast_to(b1[:, :NA], (8, NA))
    for k in range(3):
        bias_v[k] = jnp.broadcast_to(b1[:, NA + k * NS:NA + (k + 1) * NS], (8, NS))

    def first_block(j, carry):
        for jj in range(NTA):
            @pl.when(j == jj)
            def _(jj=jj):
                cp_t1(jj).wait()
                cp_t2(jj).wait()
        sl = pl.ds(pl.multiple_of(j * LANES, LANES), LANES)
        hid = _dot(xn_v[pl.ds(0, RB), :], w1a_v[:, sl]) + biasa_v[0:1, sl]
        hid = jax.nn.gelu(hid, approximate=True).astype(BF16)
        y = _dot(hid, w2a_v[sl, :])
        init = x_v[pl.ds(0, RB), :].astype(F32) + b2
        acc_v[pl.ds(0, RB), :] = jnp.where(j > 0, acc_v[pl.ds(0, RB), :], init) + y
        return carry

    lax.fori_loop(0, NTA, first_block, 0)

    for cp in cp_chunk(0):
        cp.start()

    def first_chunk(r, carry):
        @pl.when(r + 1 < nrb)
        def _():
            cp_x(r + 1).wait()

        def next_layernorm():
            zero = opaque_zero(r)
            xb = pltpu.bitcast(layernorm(jnp.minimum(r + 1, nrb - 1)), U32)
            rows = RB // 2 // KT
            zs = []
            for n in range(KT):
                blk = xb[n * rows:(n + 1) * rows]
                z = None
                for i in range(rows // 8):
                    for j in range(KT):
                        t = blk[i * 8:(i + 1) * 8, j * LANES:(j + 1) * LANES]
                        z = t if z is None else z | t
                zs.append(pltpu.bitcast(z & zero, F32))
            return zs

        ffn_block(r, w1a_v[...], w2a_v[...], b1[:, :NA], next_layernorm, True)
        return carry

    lax.fori_loop(1, nrb, first_chunk, 0)

    def later_chunk(k, carry):
        for kk in range(3):
            @pl.when(k == kk)
            def _(kk=kk):
                for cp in cp_chunk(kk):
                    cp.wait()
                for cp in (cp_chunk(kk + 1) if kk < 2 else cp_wo):
                    cp.start()

        def body(r):
            def relayout():
                zero = opaque_zero(r)
                upi = n_units // nrb
                zu = [relayout_unit(k, r * upi + uu, zero) for uu in range(upi)]
                per = upi // KT
                zs = []
                for n in range(KT):
                    z = zu[n * per]
                    for i in range(1, per):
                        z = z + zu[n * per + i]
                    zs.append(z)
                return zs

            ffn_block(r, w1s_v[k], w2s_v[k], bias_v[k, 0:1, :], relayout, False)

        _unrolled_loop(nrb, 2, body)
        return carry

    lax.fori_loop(0, 3, later_chunk, 0)

    for cp in cp_wo:
        cp.wait()

    hbuf[pl.ds(seg, M), :] = mem0_v[...].astype(F32)
    hbuf[pl.ds(0, seg), :] = xn_v[pl.ds(0, seg), :].astype(F32)

    def wtile(mi, h):
        return pltpu.bitcast(wqkv[mi, h], BF16)

    sgs, h0 = [], 0
    for sg in groups:
        gl = []
        for gn in sg:
            gl.append((h0, gn))
            h0 += gn
        sgs.append(gl)
    assert h0 == H
    NSG = len(sgs)
    V_BEFORE_S = 3
    PV_DELAY = 4
    N_SPLIT = 2
    UNROLL = 4 if n_seg % 4 == 0 else 1

    def cp_out(s):
        t0 = s * seg if isinstance(s, int) else pl.multiple_of(s * seg, seg)
        return pltpu.make_async_copy(out_v.at[pl.ds(t0, seg)], out_hbm.at[pl.ds(t0, seg)], osem.at[0])

    def step(s):
        t0 = pl.multiple_of(s * seg, seg)
        hh = hbuf[...]
        q, k, v, sc, p, rl, o = {}, {}, {}, {}, {}, {}, {}
        outp = [None] * KT

        def do_q(h):
            q[h] = _dot(hh, wtile(0, h))

        def do_k(h):
            k[h] = _dot(hh, wtile(1, h))

        def do_v(h):
            v[h] = _dot(hh, wtile(2, h))

        def half(mi, h, part):
            HD = D // 2
            w = pltpu.bitcast(wqkv[mi, h, part * (HD // 2):(part + 1) * (HD // 2), :], BF16)
            return _dot(hh[:, part * HD:(part + 1) * HD], w)

        def do_first(hs):
            qa = {h: half(0, h, 0) for h in hs}
            ka = {h: half(1, h, 0) for h in hs}
            for h in hs:
                q[h] = half(0, h, 1) + qa[h]
                k[h] = half(1, h, 1) + ka[h]

        def padcat(lst):
            n = sum(a.shape[0] for a in lst)
            return jnp.concatenate(lst + [jnp.zeros((LANES - n, Dh), F32)], axis=0).astype(BF16)

        def do_s(g):
            g0, gn = g
            qq = jnp.concatenate([q[g0 + i] for i in range(gn)], axis=0)
            sc[g] = _dot_nt(qq, padcat([k[g0 + i] for i in range(gn)]))

        def do_softmax(g):
            g0, gn = g
            R = gn * L
            t = jnp.where(maskv[0:R, :] > 0.5, sc[g] * cscale, fillv[0:R, :])
            mx = jnp.max(t, axis=-1, keepdims=True)
            pp = jnp.exp2(t - mx)
            l = jnp.sum(pp, axis=-1, keepdims=True)
            p[g] = pp
            r = _reciprocal(l, approx=True)
            rl[g] = r * (2.0 - l * r)

        def do_pv(g):
            g0, gn = g
            oo = _dot(p[g], padcat([v[g0 + i] for i in range(gn)])) * rl[g]
            for i in range(gn):
                o[g0 + i] = oo[i * L:(i + 1) * L]

        def heads(si):
            return [g0 + i for (g0, gn) in sgs[si] for i in range(gn)]

        def do_wo(si, n):
            hs = heads(si)
            oc = jnp.concatenate([o[h] for h in hs], axis=1)
            r = _dot(oc, wo_v[n, hs[0] * Dh:(hs[-1] + 1) * Dh, :])
            outp[n] = r if outp[n] is None else r + outp[n]

        def do_next_tokens():
            s1 = jnp.minimum(s + 1, n_seg - 1)
            hbuf[pl.ds(0, seg), :] = xn_v[pl.ds(pl.multiple_of(s1 * seg, seg), seg), :].astype(F32)

        tasks, pending = [], []
        for si in range(NSG):
            main = []
            hl = heads(si)
            if si == 0:
                main.append(functools.partial(do_first, hl[:N_SPLIT]))
                hl = hl[N_SPLIT:]
            for h in hl:
                main.append(functools.partial(do_q, h))
                main.append(functools.partial(do_k, h))
            vlist = [functools.partial(do_v, h) for h in heads(si)]
            main += vlist[:V_BEFORE_S]
            main += [functools.partial(do_s, g) for g in sgs[si]]
            main += [functools.partial(do_softmax, g) for g in sgs[si]]
            main += vlist[V_BEFORE_S:]
            if pending:
                main = main[:PV_DELAY] + pending + main[PV_DELAY:]
            pending = [functools.partial(do_pv, g) for g in sgs[si]]
            tasks += main
        tasks.append(do_next_tokens)
        wo_tasks = [functools.partial(do_wo, si, n) for si in range(NSG) for n in range(KT)]
        tasks += wo_tasks[:PV_DELAY] + pending + wo_tasks[PV_DELAY:]
        for t in tasks:
            t()
        res = jnp.concatenate(outp, axis=1)
        hbuf[pl.ds(seg, M), :] = res[seg:]
        out_v[pl.ds(t0, seg), :] = (acc_v[pl.ds(t0, seg), :] + res[:seg]).astype(BF16)

    def steps(i, carry):
        @pl.when(i > 0)
        def _():
            cp_out(i * UNROLL - 1).start()

        for u in range(UNROLL):
            if u > 0:
                cp_out(i * UNROLL + u - 1).start()
            step(i * UNROLL + u)
        return carry

    lax.fori_loop(0, n_seg // UNROLL, steps, 0)
    cp_out(n_seg - 1).start()
    for s in range(n_seg):
        cp_out(s).wait()


@functools.partial(jax.jit, static_argnames=("A_seg_len",))
def pallas_parallel_sum__memory_aug_recurrent_mem_tr__dense_activation_gelu__prompt_kernel(
    A_x, A_mem0, A_Wq, A_Wk, A_Wv, A_Wo, A_seg_len, B_x, B_w1, B_b1, B_w2, B_b2,
):
    del B_x
    _, S, D = A_x.shape
    _, H, Dh = A_Wq.shape
    M = A_mem0.shape[1]
    seg = int(A_seg_len)
    F = B_w1.shape[1]
    RB = 256
    NS = (F // LANES * 2 // 7) * LANES
    NA = F - 3 * NS
    groups = ((2, 2, 2, 2), (3, 3, 3, 3), (3, 3, 3, 3))
    nrb = S // RB
    KT = D // LANES
    assert Dh == LANES and D % LANES == 0 and F % LANES == 0 and NA >= 2 * LANES
    assert M % 8 == 0 and seg % 16 == 0 and 3 * (M + seg) <= LANES and S % seg == 0
    assert sum(map(sum, groups)) == H and H % 2 == 0
    assert S % RB == 0 and nrb >= 2 and (D // 16) % (nrb * KT) == 0 and RB % (16 * KT) == 0
    kern = functools.partial(_kernel, S=S, D=D, H=H, Dh=Dh, M=M, seg=seg, F=F, RB=RB, NA=NA, NS=NS,
                             groups=groups)
    hbm = pl.BlockSpec(memory_space=pl.ANY)
    out = pl.pallas_call(
        kern,
        out_shape=jax.ShapeDtypeStruct((S, D), BF16),
        in_specs=[hbm] * 10,
        out_specs=hbm,
        scratch_shapes=[
            pltpu.VMEM((S, D), BF16),
            pltpu.VMEM((S, D), BF16),
            pltpu.VMEM((S, D), F32),
            pltpu.VMEM((D, NA), BF16),
            pltpu.VMEM((NA, D), BF16),
            pltpu.VMEM((3, D, NS), BF16),
            pltpu.VMEM((3, NS, D), BF16),
            pltpu.VMEM((8, NA), F32),
            pltpu.VMEM((3, 8, NS), F32),
            pltpu.VMEM((3, D, H, Dh), BF16),
            pltpu.VMEM((3, H, D // 2, Dh), U32),
            pltpu.VMEM((D // LANES, H * Dh, LANES), BF16),
            pltpu.VMEM((M + seg, D), F32),
            pltpu.VMEM((S, D), BF16),
            pltpu.VMEM((LANES, LANES), F32),
            pltpu.VMEM((LANES, LANES), F32),
            pltpu.VMEM((M, D), BF16),
            pltpu.VMEM((F,), BF16),
            pltpu.VMEM((D,), BF16),
            pltpu.SemaphoreType.DMA((nrb + 1 + NA // LANES,)),
            pltpu.SemaphoreType.DMA((1,)),
        ],
        compiler_params=pltpu.CompilerParams(vmem_limit_bytes=110 * 1024 * 1024),
    )(A_x.reshape(S, D), A_mem0.reshape(M, D), A_Wq, A_Wk, A_Wv, A_Wo.reshape(H * Dh, D),
      B_w1, B_b1, B_w2, B_b2)
    return out.reshape(1, S, D)
```

```python
import functools
import math

import jax
import jax.numpy as jnp
import numpy as np
from jax import lax
import jax.experimental.pallas as pl
import jax.experimental.pallas.tpu as pltpu

F32 = jnp.float32
BF16 = jnp.bfloat16
U32 = jnp.uint32
LANES = 128
_reciprocal = pltpu.reciprocal if hasattr(pltpu, "reciprocal") else pl.reciprocal


def _dot(a, b):
    return lax.dot_general(a, b, (((1,), (0,)), ((), ())), preferred_element_type=F32)


def _dot_nt(a, b):
    return lax.dot_general(a, b, (((1,), (1,)), ((), ())), preferred_element_type=F32)


def _unrolled_loop(n, unroll, body):
    unroll = unroll if n % unroll == 0 else 1

    def f(i, carry):
        for k in range(unroll):
            body(i * unroll + k)
        return carry

    lax.fori_loop(0, n // unroll, f, 0)


def _kernel(x_hbm, mem0_hbm, wq_hbm, wk_hbm, wv_hbm, wo_hbm, w1_hbm, b1_hbm, w2_hbm, b2_hbm,
            out_hbm,
            x_v, xn_v, acc_v, w1a_v, w2a_v, w1s_v, w2s_v, biasa_v, bias_v, stg, wqkv, wo_v,
            hbuf, out_v, maskv, fillv, mem0_v, b1_v, b2_v, sems, osem,
            *, S, D, H, Dh, M, seg, F, RB, NA, NS, groups):
    L = M + seg
    n_seg = S // seg
    nrb = S // RB
    HP = H // 2
    KT = D // LANES
    n_units = D // 16

    s_small = nrb
    s_tile = nrb + 1
    NTA = NA // LANES

    def cp_x(r):
        r0 = r * RB if isinstance(r, int) else pl.multiple_of(r * RB, RB)
        return pltpu.make_async_copy(x_hbm.at[pl.ds(r0, RB)], x_v.at[pl.ds(r0, RB)], sems.at[r])

    def cp_t1(j):
        sl = pl.ds(j * LANES, LANES)
        return pltpu.make_async_copy(w1_hbm.at[:, sl], w1a_v.at[:, sl], sems.at[s_tile + j])

    def cp_t2(j):
        sl = pl.ds(j * LANES, LANES)
        return pltpu.make_async_copy(w2_hbm.at[sl], w2a_v.at[sl], sems.at[s_tile + j])

    def chunk_sem(k):
        return sems.at[s_tile + k % 2]

    whbm = (wq_hbm, wk_hbm, wv_hbm)

    def cp_chunk(k):
        sl = pl.ds(NA + k * NS, NS)
        return [pltpu.make_async_copy(w1_hbm.at[:, sl], w1s_v.at[k], chunk_sem(k)),
                pltpu.make_async_copy(w2_hbm.at[sl], w2s_v.at[k], chunk_sem(k)),
                pltpu.make_async_copy(whbm[k], stg.at[k], chunk_sem(k))]

    cp_wo = [pltpu.make_async_copy(wo_hbm.at[:, pl.ds(n * LANES, LANES)], wo_v.at[n], chunk_sem(3))
             for n in range(KT)]
    cp_small = [pltpu.make_async_copy(src, dst, sems.at[s_small])
                for src, dst in ((b1_hbm, b1_v), (b2_hbm, b2_v), (mem0_hbm, mem0_v))]

    cp_x(0).start()
    cp_x(1).start()
    for cp in cp_small:
        cp.start()
    for j in range(NTA):
        cp_t1(j).start()
        cp_t2(j).start()
    for r in range(2, nrb):
        cp_x(r).start()

    ri = lax.broadcasted_iota(jnp.int32, (LANES, LANES), 0)
    ci = lax.broadcasted_iota(jnp.int32, (LANES, LANES), 1)
    rb_ = (ri >= L).astype(jnp.int32) + (ri >= 2 * L) + (ri >= 3 * L)
    cb_ = (ci >= L).astype(jnp.int32) + (ci >= 2 * L) + (ci >= 3 * L)
    rw, cw = ri - L * rb_, ci - L * cb_
    same = rb_ == cb_
    valid = same & ((rw >= seg) | (cw >= seg) | (rw >= cw))
    log2e = math.log2(math.e)
    maskv[...] = valid.astype(F32)
    fillv[...] = jnp.where(same, -1e9 * log2e, -jnp.inf).astype(F32)
    cscale = (Dh ** -0.5) * log2e

    def relayout_unit(mi, u, zero):
        s32 = stg.at[mi].bitcast(U32)
        d0 = pl.multiple_of(u * 16, 16)
        X = s32[pl.ds(d0, 16)].reshape(8, 2, HP, Dh)
        A = X[:, 0]
        B = X[:, 1]
        E = (A & np.uint32(0xFFFF)) | (B << 16)
        O = (A >> 16) | (B & np.uint32(0xFFFF0000))
        Et = jnp.swapaxes(E, 0, 1)
        Ot = jnp.swapaxes(O, 0, 1)
        p0 = pl.multiple_of(u * 8, 8)
        z = None
        for j in range(HP):
            wqkv[mi, 2 * j, pl.ds(p0, 8), :] = Et[j]
            wqkv[mi, 2 * j + 1, pl.ds(p0, 8), :] = Ot[j]
            zz = Et[j] | Ot[j]
            z = zz if z is None else z | zz
        return pltpu.bitcast(z & zero, F32)

    def layernorm_rows(r0, n):
        xf = x_v[pl.ds(r0, n), :].astype(F32)
        m = jnp.mean(xf, axis=-1, keepdims=True)
        xc = xf - m
        var = jnp.mean(xc * xc, axis=-1, keepdims=True)
        xn = (xc * lax.rsqrt(var + 1e-5)).astype(BF16)
        xn_v[pl.ds(r0, n), :] = xn
        return xn

    def layernorm(r):
        return layernorm_rows(pl.multiple_of(r * RB, RB), RB)

    def opaque_zero(r):
        return jnp.full((8, LANES), r >> 20, jnp.int32).astype(U32)

    def ffn_block(r, w1, w2, bias, side_work, first):
        r0 = pl.multiple_of(r * RB, RB)
        xn = xn_v[pl.ds(r0, RB), :]
        hid = _dot(xn, w1) + bias
        hid = jax.nn.gelu(hid, approximate=True).astype(BF16)
        y = _dot(hid, w2)
        zs = side_work()
        y = jnp.concatenate([y[:8] + jnp.concatenate(zs, axis=1), y[8:]], axis=0)
        if first:
            xf = x_v[pl.ds(r0, RB), :].astype(F32)
            acc_v[pl.ds(r0, RB), :] = y + (xf + b2)
        else:
            acc_v[pl.ds(r0, RB), :] += y

    def first_layernorms(i, carry):
        for rr in range(2):
            @pl.when(i == 2 * rr)
            def _(rr=rr):
                cp_x(rr).wait()
        layernorm_rows(pl.multiple_of(i * (RB // 2), RB // 2), RB // 2)
        return carry

    lax.fori_loop(0, 4, first_layernorms, 0)
    for cp in cp_small:
        cp.wait()
    b1 = b1_v[...].astype(F32).reshape(1, F)
    b2 = b2_v[...].astype(F32).reshape(1, D)
    biasa_v[...] = jnp.broadcast_to(b1[:, :NA], (8, NA))
    for k in range(3):
        bias_v[k] = jnp.broadcast_to(b1[:, NA + k * NS:NA + (k + 1) * NS], (8, NS))

    acc_v[pl.ds(0, RB), :] = x_v[pl.ds(0, RB), :].astype(F32) + b2

    def first_block(j, carry):
        for jj in range(NTA):
            @pl.when(j == jj)
            def _(jj=jj):
                cp_t1(jj).wait()
                cp_t2(jj).wait()
        sl = pl.ds(pl.multiple_of(j * LANES, LANES), LANES)
        hid = _dot(xn_v[pl.ds(0, RB), :], w1a_v[:, sl]) + biasa_v[0:1, sl]
        hid = jax.nn.gelu(hid, approximate=True).astype(BF16)
        y = _dot(hid, w2a_v[sl, :])
        acc_v[pl.ds(0, RB), :] += y
        return carry

    lax.fori_loop(0, NTA, first_block, 0)

    for cp in cp_chunk(0):
        cp.start()

    def first_chunk(r, carry):
        @pl.when(r + 1 < nrb)
        def _():
            cp_x(r + 1).wait()

        def next_layernorm():
            zero = opaque_zero(r)
            xb = pltpu.bitcast(layernorm(jnp.minimum(r + 1, nrb - 1)), U32)
            rows = RB // 2 // KT
            zs = []
            for n in range(KT):
                blk = xb[n * rows:(n + 1) * rows]
                z = None
                for i in range(rows // 8):
                    for j in range(KT):
                        t = blk[i * 8:(i + 1) * 8, j * LANES:(j + 1) * LANES]
                        z = t if z is None else z | t
                zs.append(pltpu.bitcast(z & zero, F32))
            return zs

        ffn_block(r, w1a_v[...], w2a_v[...], b1[:, :NA], next_layernorm, True)
        return carry

    lax.fori_loop(1, nrb, first_chunk, 0)

    def later_chunk(k, carry):
        for kk in range(3):
            @pl.when(k == kk)
            def _(kk=kk):
                for cp in cp_chunk(kk):
                    cp.wait()
                for cp in (cp_chunk(kk + 1) if kk < 2 else cp_wo):
                    cp.start()

        def body(r):
            def relayout():
                zero = opaque_zero(r)
                upi = n_units // nrb
                zu = [relayout_unit(k, r * upi + uu, zero) for uu in range(upi)]
                per = upi // KT
                zs = []
                for n in range(KT):
                    z = zu[n * per]
                    for i in range(1, per):
                        z = z + zu[n * per + i]
                    zs.append(z)
                return zs

            ffn_block(r, w1s_v[k], w2s_v[k], bias_v[k, 0:1, :], relayout, False)

        _unrolled_loop(nrb, 2, body)
        return carry

    lax.fori_loop(0, 3, later_chunk, 0)

    for cp in cp_wo:
        cp.wait()

    hbuf[pl.ds(seg, M), :] = mem0_v[...].astype(F32)
    hbuf[pl.ds(0, seg), :] = xn_v[pl.ds(0, seg), :].astype(F32)

    def wtile(mi, h):
        return pltpu.bitcast(wqkv[mi, h], BF16)

    sgs, h0 = [], 0
    for sg in groups:
        gl = []
        for gn in sg:
            gl.append((h0, gn))
            h0 += gn
        sgs.append(gl)
    assert h0 == H
    NSG = len(sgs)
    V_BEFORE_S = 3
    PV_DELAY = 4
    N_SPLIT = 2
    UNROLL = 4 if n_seg % 4 == 0 else 1

    def cp_out(s):
        t0 = s * seg if isinstance(s, int) else pl.multiple_of(s * seg, seg)
        return pltpu.make_async_copy(out_v.at[pl.ds(t0, seg)], out_hbm.at[pl.ds(t0, seg)], osem.at[0])

    def step(s):
        t0 = pl.multiple_of(s * seg, seg)
        hh = hbuf[...]
        q, k, v, sc, p, rl, o = {}, {}, {}, {}, {}, {}, {}
        outp = [None] * KT

        def do_q(h):
            q[h] = _dot(hh, wtile(0, h))

        def do_k(h):
            k[h] = _dot(hh, wtile(1, h))

        def do_v(h):
            v[h] = _dot(hh, wtile(2, h))

        def half(mi, h, part):
            HD = D // 2
            w = pltpu.bitcast(wqkv[mi, h, part * (HD // 2):(part + 1) * (HD // 2), :], BF16)
            return _dot(hh[:, part * HD:(part + 1) * HD], w)

        def do_first(hs):
            qa = {h: half(0, h, 0) for h in hs}
            ka = {h: half(1, h, 0) for h in hs}
            for h in hs:
                q[h] = half(0, h, 1) + qa[h]
                k[h] = half(1, h, 1) + ka[h]

        def padcat(lst):
            n = sum(a.shape[0] for a in lst)
            return jnp.concatenate(lst + [jnp.zeros((LANES - n, Dh), F32)], axis=0).astype(BF16)

        def do_s(g):
            g0, gn = g
            qq = jnp.concatenate([q[g0 + i] for i in range(gn)], axis=0)
            sc[g] = _dot_nt(qq, padcat([k[g0 + i] for i in range(gn)]))

        def do_softmax(g):
            g0, gn = g
            R = gn * L
            t = jnp.where(maskv[0:R, :] > 0.5, sc[g] * cscale, fillv[0:R, :])
            mx = jnp.max(t, axis=-1, keepdims=True)
            pp = jnp.exp2(t - mx)
            l = jnp.sum(pp, axis=-1, keepdims=True)
            p[g] = pp
            r = _reciprocal(l, approx=True)
            rl[g] = r * (2.0 - l * r)

        def do_pv(g):
            g0, gn = g
            oo = _dot(p[g], padcat([v[g0 + i] for i in range(gn)])) * rl[g]
            for i in range(gn):
                o[g0 + i] = oo[i * L:(i + 1) * L]

        def heads(si):
            return [g0 + i for (g0, gn) in sgs[si] for i in range(gn)]

        def do_wo(si, n):
            hs = heads(si)
            oc = jnp.concatenate([o[h] for h in hs], axis=1)
            r = _dot(oc, wo_v[n, hs[0] * Dh:(hs[-1] + 1) * Dh, :])
            outp[n] = r if outp[n] is None else r + outp[n]

        def do_next_tokens():
            s1 = jnp.minimum(s + 1, n_seg - 1)
            hbuf[pl.ds(0, seg), :] = xn_v[pl.ds(pl.multiple_of(s1 * seg, seg), seg), :].astype(F32)

        tasks, pending = [], []
        for si in range(NSG):
            main = []
            hl = heads(si)
            if si == 0:
                main.append(functools.partial(do_first, hl[:N_SPLIT]))
                hl = hl[N_SPLIT:]
            for h in hl:
                main.append(functools.partial(do_q, h))
                main.append(functools.partial(do_k, h))
            vlist = [functools.partial(do_v, h) for h in heads(si)]
            main += vlist[:V_BEFORE_S]
            main += [functools.partial(do_s, g) for g in sgs[si]]
            main += [functools.partial(do_softmax, g) for g in sgs[si]]
            main += vlist[V_BEFORE_S:]
            if pending:
                main = main[:PV_DELAY] + pending + main[PV_DELAY:]
            pending = [functools.partial(do_pv, g) for g in sgs[si]]
            tasks += main
        tasks.append(do_next_tokens)
        wo_tasks = [functools.partial(do_wo, si, n) for si in range(NSG) for n in range(KT)]
        tasks += wo_tasks[:PV_DELAY] + pending + wo_tasks[PV_DELAY:]
        for t in tasks:
            t()
        res = jnp.concatenate(outp, axis=1)
        hbuf[pl.ds(seg, M), :] = res[seg:]
        out_v[pl.ds(t0, seg), :] = (acc_v[pl.ds(t0, seg), :] + res[:seg]).astype(BF16)

    def steps(i, carry):
        @pl.when(i > 0)
        def _():
            cp_out(i * UNROLL - 1).start()

        for u in range(UNROLL):
            if u > 0:
                cp_out(i * UNROLL + u - 1).start()
            step(i * UNROLL + u)
        return carry

    lax.fori_loop(0, n_seg // UNROLL, steps, 0)
    cp_out(n_seg - 1).start()
    for s in range(n_seg):
        cp_out(s).wait()


@functools.partial(jax.jit, static_argnames=("A_seg_len",))
def pallas_parallel_sum__memory_aug_recurrent_mem_tr__dense_activation_gelu__prompt_kernel(
    A_x, A_mem0, A_Wq, A_Wk, A_Wv, A_Wo, A_seg_len, B_x, B_w1, B_b1, B_w2, B_b2,
):
    del B_x
    _, S, D = A_x.shape
    _, H, Dh = A_Wq.shape
    M = A_mem0.shape[1]
    seg = int(A_seg_len)
    F = B_w1.shape[1]
    RB = 256
    NS = (F // LANES * 2 // 7) * LANES
    NA = F - 3 * NS
    groups = ((2, 2, 2, 2), (3, 3, 3, 3), (3, 3, 3, 3))
    nrb = S // RB
    KT = D // LANES
    assert Dh == LANES and D % LANES == 0 and F % LANES == 0 and NA >= 2 * LANES
    assert M % 8 == 0 and seg % 16 == 0 and 3 * (M + seg) <= LANES and S % seg == 0
    assert sum(map(sum, groups)) == H and H % 2 == 0
    assert S % RB == 0 and nrb >= 2 and (D // 16) % (nrb * KT) == 0 and RB % (16 * KT) == 0
    kern = functools.partial(_kernel, S=S, D=D, H=H, Dh=Dh, M=M, seg=seg, F=F, RB=RB, NA=NA, NS=NS,
                             groups=groups)
    hbm = pl.BlockSpec(memory_space=pl.ANY)
    out = pl.pallas_call(
        kern,
        out_shape=jax.ShapeDtypeStruct((S, D), BF16),
        in_specs=[hbm] * 10,
        out_specs=hbm,
        scratch_shapes=[
            pltpu.VMEM((S, D), BF16),
            pltpu.VMEM((S, D), BF16),
            pltpu.VMEM((S, D), F32),
            pltpu.VMEM((D, NA), BF16),
            pltpu.VMEM((NA, D), BF16),
            pltpu.VMEM((3, D, NS), BF16),
            pltpu.VMEM((3, NS, D), BF16),
            pltpu.VMEM((8, NA), F32),
            pltpu.VMEM((3, 8, NS), F32),
            pltpu.VMEM((3, D, H, Dh), BF16),
            pltpu.VMEM((3, H, D // 2, Dh), U32),
            pltpu.VMEM((D // LANES, H * Dh, LANES), BF16),
            pltpu.VMEM((M + seg, D), F32),
            pltpu.VMEM((S, D), BF16),
            pltpu.VMEM((LANES, LANES), F32),
            pltpu.VMEM((LANES, LANES), F32),
            pltpu.VMEM((M, D), BF16),
            pltpu.VMEM((F,), BF16),
            pltpu.VMEM((D,), BF16),
            pltpu.SemaphoreType.DMA((nrb + 1 + NA // LANES,)),
            pltpu.SemaphoreType.DMA((1,)),
        ],
        compiler_params=pltpu.CompilerParams(vmem_limit_bytes=110 * 1024 * 1024),
    )(A_x.reshape(S, D), A_mem0.reshape(M, D), A_Wq, A_Wk, A_Wv, A_Wo.reshape(H * Dh, D),
      B_w1, B_b1, B_w2, B_b2)
    return out.reshape(1, S, D)
```
